```python
import os as _os
_os.environ.setdefault("JAX_PLATFORMS", "cpu")
import jax
import jax.numpy as jnp

def _softmax(x, axis=-1):
    return jax.nn.softmax(x, axis=axis)
def _gelu(x):
    return jax.nn.gelu(x, approximate=True)
def _silu(x):
    return jax.nn.silu(x)
def _sigmoid(x):
    return jax.nn.sigmoid(x)
def _layernorm(x, axis=-1, eps=1e-5):
    m = jnp.mean(x, axis=axis, keepdims=True)
    v = jnp.var(x, axis=axis, keepdims=True)
    return (x - m) / jnp.sqrt(v + eps)
def _scatter_add(tgt, idx, src, axis=0):
    return tgt.at[idx].add(src)
def _segment_sum(src, seg, n):
    return jax.ops.segment_sum(src, seg, n)
class _Rng:
    def __init__(self, key):
        self._k = key
    def _next(self):
        self._k, sub = jax.random.split(self._k)
        return sub
    def normal(self, shape):
        return jax.random.normal(self._next(), shape, dtype=jnp.bfloat16)
    def randint(self, lo, hi, shape):
        return jax.random.randint(self._next(), shape, lo, hi, dtype=jnp.int32)
    def uniform(self, shape, lo=0.0, hi=1.0):
        return jax.random.uniform(self._next(), shape, jnp.bfloat16, lo, hi)
    def permutation(self, n):
        return jax.random.permutation(self._next(), n)


kernel_name = 'interleave_layers__grouped_kv_mqa__dense_activation_relu__prompt'

def setup_inputs():
    _rng = _Rng(jax.random.key(int.from_bytes(__import__("os").urandom(4), "little")))
    _w = (lambda a: (lambda t: t.astype(jnp.bfloat16) if jnp.issubdtype(t.dtype, jnp.floating) else t)(jnp.asarray(a)))
    def _A_setup():
        B, S, D, H = 1, 2048, 448, 16
        Dh = D // H
        return {
            "x": _w((lambda *s: _rng.normal(s) * 0.05)(B, S, D)),
            "wq": _w((lambda *s: _rng.normal(s) * 0.05)(D, H * Dh)),
            "wk": _w((lambda *s: _rng.normal(s) * 0.05)(D, Dh)),
            "wv": _w((lambda *s: _rng.normal(s) * 0.05)(D, Dh)),
            "wo": _w((lambda *s: _rng.normal(s) * 0.05)(H * Dh, D)),
        }
    _A_in = _A_setup()

    def _B_setup():
        B, S, D, Dff = 1, 2048, 448, 1792
        return {
            "x": _w((lambda *s: _rng.normal(s) * 0.05)(B, S, D)),
            "w1": _w((lambda *s: _rng.normal(s) * 0.05)(D, Dff)),
            "w2": _w((lambda *s: _rng.normal(s) * 0.05)(Dff, D)),
        }
    _B_in = _B_setup()

    return {
        "A_x": _A_in["x"],
        "A_wq": _A_in["wq"],
        "A_wk": _A_in["wk"],
        "A_wv": _A_in["wv"],
        "A_wo": _A_in["wo"],
        "B_x": _B_in["x"],
        "B_w1": _B_in["w1"],
        "B_w2": _B_in["w2"],
    }

def reference(A_x, A_wq, A_wk, A_wv, A_wo, B_x, B_w1, B_w2):
    def _A_ref(x, wq, wk, wv, wo):
        B, S, D = x.shape
        H = 16
        Dh = D // H
        q = (lambda x, *d: x.transpose(*d))((x @ wq).reshape(B, S, H, Dh), 0, 2, 1, 3)
        k = x @ wk
        v = x @ wv
        scores = jnp.einsum("bhqd,bkd->bhqk", q, k) * (Dh ** -0.5)
        p = _softmax(scores, axis=-1)
        o = jnp.einsum("bhqk,bkd->bhqd", p, v)
        return (lambda x, *d: x.transpose(*d))(o, 0, 2, 1, 3).reshape(B, S, H * Dh) @ wo

    def _B_ref(x, w1, w2):
        h = jnp.einsum("bsd,df->bsf", x, w1)
        zero = jnp.zeros_like(h)
        h = jnp.maximum(h, zero)
        return jnp.einsum("bsf,fd->bsd", h, w2)

    x = A_x
    x = x + _A_ref(_layernorm(x, axis=-1), A_wq, A_wk, A_wv, A_wo)
    x = x + _B_ref(_layernorm(x, axis=-1), B_w1, B_w2)
    x = x + _A_ref(_layernorm(x, axis=-1), A_wq, A_wk, A_wv, A_wo)
    x = x + _B_ref(_layernorm(x, axis=-1), B_w1, B_w2)
    return x
```

```python
import functools
import math

import jax
import jax.numpy as jnp
from jax import lax
from jax.experimental import pallas as pl
from jax.experimental.pallas import tpu as pltpu

f32 = jnp.float32
bf16 = jnp.bfloat16

S = 2048
D = 448
H = 16
DH = 28
DP = 32
DFF = 1792
TB = 512
NB = S // TB
CK = 256
NC = S // CK
NT = H * NB
TPB = 4
SUB = 256
EPS = 1e-5
QSCALE = (DH ** -0.5) * math.log2(math.e)
NQ = H * DP
NQKV = NQ + 2 * DP

NT_DIMS = (((1,), (1,)), ((), ()))
TN_DIMS = (((0,), (0,)), ((), ()))


def _ln_t(x):
    mu = jnp.mean(x, axis=0, keepdims=True)
    xc = x - mu
    var = jnp.mean(xc * xc, axis=0, keepdims=True)
    return (xc * lax.rsqrt(var + EPS)).astype(bf16)


def _tree_max8(s):
    r = s.shape[0]
    while r > 8:
        r //= 2
        s = jnp.maximum(s[:r], s[r:])
    return s


def _kernel(x_hbm, wq_hbm, wkt_hbm, wvt_hbm, wo_hbm, w1_hbm, w2t_hbm, out_hbm,
            xin, wq_v, wkt_v, wvt_v, wo_v, w1_v, w2t_v,
            xres, wqkv_t, wo_t, w1_t, k_s, qt_s, vt_s, ot_s, s0, s1, m0, m1, outb,
            sem_in, sem_x, sem_out):
    cps = []
    for i, (src, dst) in enumerate([(wq_hbm, wq_v), (wkt_hbm, wkt_v), (wvt_hbm, wvt_v)]):
        cp = pltpu.make_async_copy(src, dst, sem_in.at[i]); cp.start(); cps.append(cp)
    xcps = []
    for b in range(NB):
        cp = pltpu.make_async_copy(x_hbm.at[0, :, pl.ds(b * TB, TB)], xin.at[b], sem_x.at[b])
        cp.start(); xcps.append(cp)
    late = []
    for i, (src, dst) in enumerate([(wo_hbm, wo_v), (w1_hbm, w1_v), (w2t_hbm, w2t_v)]):
        cp = pltpu.make_async_copy(src, dst, sem_in.at[3 + i]); cp.start(); late.append(cp)

    for cp in cps:
        cp.wait()
    r = lax.broadcasted_iota(jnp.int32, (NQ, D), 0)
    c = lax.broadcasted_iota(jnp.int32, (NQ, D), 1)
    rh = r // DP
    rd = r - rh * DP
    esel = jnp.where((c == rh * DH + rd) & (rd < DH), 1.0, 0.0).astype(bf16)
    wqkv_t[0:NQ, :] = lax.dot_general(esel, wq_v[...], NT_DIMS, preferred_element_type=f32).astype(bf16)
    r2 = lax.broadcasted_iota(jnp.int32, (DP, DH), 0)
    c2 = lax.broadcasted_iota(jnp.int32, (DP, DH), 1)
    e2 = jnp.where(r2 == c2, 1.0, 0.0).astype(bf16)
    wqkv_t[NQ:NQ + DP, :] = jnp.dot(e2, wvt_v[...], preferred_element_type=f32).astype(bf16)
    wqkv_t[NQ + DP:NQKV, :] = jnp.dot(e2, wkt_v[...], preferred_element_type=f32).astype(bf16)

    def qkv_sub(b, u, xs):
        xn = _ln_t(xs)
        qkv = jnp.dot(wqkv_t[...], xn, preferred_element_type=f32)
        qt_s[b, :, u * SUB:(u + 1) * SUB] = (qkv[0:NQ] * QSCALE).astype(bf16)
        v = qkv[NQ:NQ + DP]
        rr = lax.broadcasted_iota(jnp.int32, (DP, SUB), 0)
        v = jnp.where(rr == DH, 1.0, v)
        vt_s[b, :, u * SUB:(u + 1) * SUB] = v.astype(bf16)
        row0 = pl.multiple_of(b * TB + u * SUB, SUB)
        k_s[pl.ds(row0, SUB), :] = qkv[NQ + DP:].T.astype(bf16)

    for b in range(NB):
        xcps[b].wait()
        for u in range(TB // SUB):
            xs = xin[b, :, u * SUB:(u + 1) * SUB].astype(f32)
            xres[b, :, u * SUB:(u + 1) * SUB] = xs
            qkv_sub(b, u, xs)

    for cp in late:
        cp.wait()
    wo_t[...] = lax.dot_general(wo_v[...], esel, (((0,), (1,)), ((), ())), preferred_element_type=f32).astype(bf16)
    w1_t[...] = w1_v[...].T

    def idx(t):
        return t % H, t // H

    def ab(ta, sa, ma, tb, sb, mb):
        if ta is not None:
            ha, qa = idx(ta)
            w = qt_s[qa, pl.ds(pl.multiple_of(ha * DP, DP), DP), :]
        if tb is not None:
            mbv = mb[0:1, :]
        m8 = None
        acc = None
        for c in range(NC):
            if ta is not None:
                s = jnp.dot(k_s[c * CK:(c + 1) * CK, :], w, preferred_element_type=f32)
                sa[c * CK:(c + 1) * CK, :] = s
                mc = _tree_max8(s)
                m8 = mc if m8 is None else jnp.maximum(m8, mc)
            if tb is not None:
                p = jnp.exp2(sb[c * CK:(c + 1) * CK, :] - mbv).astype(bf16)
                cb, co = divmod(c * CK, TB)
                d = jnp.dot(vt_s[cb, :, co:co + CK], p, preferred_element_type=f32)
                acc = d if acc is None else acc + d
        if ta is not None:
            ma[...] = jnp.broadcast_to(jnp.max(m8, axis=0, keepdims=True), (8, TB))
        if tb is not None:
            hb, qb = idx(tb)
            inv = 1.0 / acc[DH:DH + 1, :]
            ot_s[qb, pl.ds(pl.multiple_of(hb * DP, DP), DP), :] = (acc * inv).astype(bf16)

    def attention():
        ab(0, s0, m0, None, None, None)

        def body(j, carry):
            for u in range(0, TPB, 2):
                t = TPB * j + u
                ab(t + 1, s1, m1, t, s0, m0)
                ab(jnp.minimum(t + 2, NT - 1), s0, m0, t + 1, s1, m1)
            return carry
        lax.fori_loop(0, NT // TPB, body, 0)

    def dense(b, last):
        nsub = TB // SUB
        x1 = []
        for u in range(nsub):
            o = jnp.dot(wo_t[...], ot_s[b, :, u * SUB:(u + 1) * SUB], preferred_element_type=f32)
            x1.append(xres[b, :, u * SUB:(u + 1) * SUB] + o)
        hs = []
        for u in range(nsub):
            hs.append(jnp.maximum(jnp.dot(w1_t[...], _ln_t(x1[u]), preferred_element_type=f32), 0.0).astype(bf16))
        x2 = []
        for u in range(nsub):
            x2.append(x1[u] + jnp.dot(w2t_v[...], hs[u], preferred_element_type=f32))
        for u in range(nsub):
            if last:
                outb[b, :, u * SUB:(u + 1) * SUB] = x2[u].astype(bf16)
            else:
                xres[b, :, u * SUB:(u + 1) * SUB] = x2[u]
                qkv_sub(b, u, x2[u])
        if last:
            c0 = pl.multiple_of(b * TB, TB)
            pltpu.make_async_copy(outb.at[b], out_hbm.at[0, :, pl.ds(c0, TB)], sem_out.at[b]).start()

    def layer(l, carry):
        attention()

        @pl.when(l == 0)
        def _():
            def body(b, c):
                dense(b, False)
                return c
            lax.fori_loop(0, NB, body, 0)

        @pl.when(l == 1)
        def _():
            def body(b, c):
                dense(b, True)
                return c
            lax.fori_loop(0, NB, body, 0)
        return carry

    lax.fori_loop(0, 2, layer, 0)
    for b in range(NB):
        pltpu.make_async_copy(outb.at[b], out_hbm.at[0, :, pl.ds(b * TB, TB)], sem_out.at[b]).wait()


@jax.jit
def pallas_interleave_layers__grouped_kv_mqa__dense_activation_relu__prompt_kernel(
    A_x, A_wq, A_wk, A_wv, A_wo, B_x, B_w1, B_w2,
):
    del B_x
    hbm_spec = pl.BlockSpec(memory_space=pltpu.HBM)
    scratch = [
        pltpu.VMEM((NB, D, TB), bf16),
        pltpu.VMEM((D, D), bf16),
        pltpu.VMEM((DH, D), bf16),
        pltpu.VMEM((DH, D), bf16),
        pltpu.VMEM((D, D), bf16),
        pltpu.VMEM((D, DFF), bf16),
        pltpu.VMEM((D, DFF), bf16),
        pltpu.VMEM((NB, D, TB), f32),
        pltpu.VMEM((NQKV, D), bf16),
        pltpu.VMEM((D, NQ), bf16),
        pltpu.VMEM((DFF, D), bf16),
        pltpu.VMEM((S, DP), bf16),
        pltpu.VMEM((NB, NQ, TB), bf16),
        pltpu.VMEM((NB, DP, TB), bf16),
        pltpu.VMEM((NB, NQ, TB), bf16),
        pltpu.VMEM((S, TB), f32),
        pltpu.VMEM((S, TB), f32),
        pltpu.VMEM((8, TB), f32),
        pltpu.VMEM((8, TB), f32),
        pltpu.VMEM((NB, D, TB), bf16),
        pltpu.SemaphoreType.DMA((6,)),
        pltpu.SemaphoreType.DMA((NB,)),
        pltpu.SemaphoreType.DMA((NB,)),
    ]
    out_t = pl.pallas_call(
        _kernel,
        out_shape=jax.ShapeDtypeStruct((1, D, S), A_x.dtype),
        in_specs=[hbm_spec] * 7,
        out_specs=hbm_spec,
        scratch_shapes=scratch,
        compiler_params=pltpu.CompilerParams(vmem_limit_bytes=100 * 1024 * 1024),
        name="fused_layers",
    )(jnp.transpose(A_x, (0, 2, 1)), A_wq, A_wk.T, A_wv.T, A_wo, B_w1, B_w2.T)
    return jnp.transpose(out_t, (0, 2, 1))
```

```python
import functools
import math

import jax
import jax.numpy as jnp
from jax import lax
from jax.experimental import pallas as pl
from jax.experimental.pallas import tpu as pltpu

f32 = jnp.float32
bf16 = jnp.bfloat16

S = 2048
D = 448
H = 16
DH = 28
DP = 32
DFF = 1792
TB = 512
NB = S // TB
CKA = 128
CKB = 256
NCA = S // CKA
NCB = S // CKB
NT = H * NB
TPB = 9
SUB = 256
NSUB = TB // SUB
EPS = 1e-5
SKEW = 128
WAIT_U = 1
QSCALE = (DH ** -0.5) * math.log2(math.e)
NQ = H * DP
NQKV = D + 2 * DP
NIT = (NT - 1) // TPB
W1C = DFF // NIT

NT_DIMS = (((1,), (1,)), ((), ()))


def _ln_t(x):
    mu = jnp.mean(x, axis=0, keepdims=True)
    xc = x - mu
    var = jnp.mean(xc * xc, axis=0, keepdims=True)
    return (xc * lax.rsqrt(var + EPS)).astype(bf16)


def _tree_max8(s):
    r = s.shape[0]
    while r > 8:
        r //= 2
        s = jnp.maximum(s[:r], s[r:])
    return s


def _kernel(x_hbm, wq_hbm, wkt_hbm, wvt_hbm, wo_hbm, w1_hbm, w2t_hbm, out_hbm,
            xin, wq_v, wkt_v, wvt_v, wo_v, w1_v, w2t_v,
            xres, wqkv_t, wo_t, w1_t, k_s, qt_s, vt_s, ot_s, s0, s1, s2, m0, m1, m2, outb,
            sem_in, sem_x, sem_out):
    sbuf = (s0, s1, s2)
    mbuf = (m0, m1, m2)
    early = []
    for i, (src, dst) in enumerate([(wq_hbm, wq_v), (wkt_hbm, wkt_v), (wvt_hbm, wvt_v)]):
        cp = pltpu.make_async_copy(src, dst, sem_in.at[i]); cp.start(); early.append(cp)
    xcps = [pltpu.make_async_copy(x_hbm.at[0, :, pl.ds(b * TB, TB)], xin.at[b], sem_x.at[b]) for b in range(NB)]
    for cp in xcps:
        cp.start()
    late = [pltpu.make_async_copy(wo_hbm, wo_v, sem_in.at[3]),
            pltpu.make_async_copy(w1_hbm, w1_v, sem_in.at[4]),
            pltpu.make_async_copy(w2t_hbm, w2t_v, sem_in.at[5])]

    for b in range(NB):
        xres[b] = jnp.zeros((D, TB), f32)
    for cp in early:
        cp.wait()
    wqkv_t[0:D, :] = wq_v[...].T
    zpad = jnp.zeros((DP - DH, D), bf16)
    wqkv_t[D:D + DP, :] = jnp.concatenate([wvt_v[...], zpad], axis=0)
    wqkv_t[D + DP:NQKV, :] = jnp.concatenate([wkt_v[...], zpad], axis=0)
    for cp in late:
        cp.start()

    def p1(l):
        order = [(b, u) for b in range(NB) for u in range(NSUB)]

        @pl.when(l == 0)
        def _():
            for cp in xcps:
                cp.wait()

        for i, (b, u) in enumerate(order):
            cols = slice(u * SUB, (u + 1) * SUB)
            xs = jnp.where(l == 0, xin[b, :, cols].astype(f32), xres[b, :, cols])
            xres[b, :, cols] = xs
            qkv_sub(b, u, xs)

    def qkv_sub(b, u, xs):
        cols = slice(u * SUB, (u + 1) * SUB)
        xn = _ln_t(xs)
        qkv = jnp.dot(wqkv_t[...], xn, preferred_element_type=f32)
        for h in range(H):
            qt_s[b, h * DP:(h + 1) * DP, cols] = (qkv[h * DH:h * DH + DP] * QSCALE).astype(bf16)
        v = qkv[D:D + DP]
        rr = lax.broadcasted_iota(jnp.int32, (DP, SUB), 0)
        v = jnp.where(rr == DH, 1.0, v)
        vt_s[b, :, cols] = v.astype(bf16)
        row0 = b * TB + u * SUB
        k_s[row0:row0 + SUB, :] = qkv[D + DP:].T.astype(bf16)

    def idx(t):
        return t % H, t // H

    def a_items(ta, sa, ma):
        st = {}

        def chunk(c):
            def f():
                if c == 0:
                    ha, qa = idx(ta)
                    st["w"] = qt_s[qa, pl.ds(pl.multiple_of(ha * DP, DP), DP), :]
                s = jnp.dot(k_s[c * CKA:(c + 1) * CKA, :], st["w"], preferred_element_type=f32)
                sa[c * CKA:(c + 1) * CKA, :] = s
                mc = _tree_max8(s)
                st["m"] = mc if c == 0 else jnp.maximum(st["m"], mc)
                if c == NCA - 1:
                    ma[...] = jnp.broadcast_to(jnp.max(st["m"], axis=0, keepdims=True), (8, TB))
            return f
        return [chunk(c) for c in range(NCA)]

    def b_items(tb, sb, mb):
        st = {}

        def chunk(c):
            def f():
                if c == 0:
                    st["m"] = mb[0:1, :]
                p = jnp.exp2(sb[c * CKB:(c + 1) * CKB, :] - st["m"]).astype(bf16)
                cb, co = divmod(c * CKB, TB)
                d = jnp.dot(vt_s[cb, :, co:co + CKB], p, preferred_element_type=f32)
                st["acc"] = d if c == 0 else st["acc"] + d
                if c == NCB - 1:
                    hb, qb = idx(tb)
                    acc = st["acc"]
                    inv = 1.0 / acc[DH:DH + 1, :]
                    ot_s[qb, pl.ds(pl.multiple_of(hb * DP, DP), DP), :] = (acc * inv).astype(bf16)
            return f
        return [chunk(c) for c in range(NCB)]

    def attn_loop():
        def body(j, carry):
            ai, bi = [], []
            for u in range(TPB):
                t = TPB * j + u
                ai += a_items(t + 1, sbuf[(u + 1) % 3], mbuf[(u + 1) % 3])
                bi += b_items(t, sbuf[u % 3], mbuf[u % 3])
            seq = [(i * CKA, 0, f) for i, f in enumerate(ai)] + [(i * CKB + SKEW, 1, f) for i, f in enumerate(bi)]
            for _, _, f in sorted(seq, key=lambda e: e[:2]):
                f()
            c0 = pl.multiple_of(j * W1C, W1C)
            w1_t[pl.ds(c0, W1C), :] = w1_v[:, pl.ds(c0, W1C)].T
            return carry
        lax.fori_loop(0, NIT, body, 0)

    def dense_items(b):
        st = {}

        def proj(u):
            def f():
                cols = slice(u * SUB, (u + 1) * SUB)
                o = jnp.dot(wo_t[...], ot_s[b, :, cols], preferred_element_type=f32)
                st["x1", u] = xres[b, :, cols] + o
            return f

        def ff1(u):
            def f():
                st["h", u] = jnp.maximum(
                    jnp.dot(w1_t[...], _ln_t(st["x1", u]), preferred_element_type=f32), 0.0).astype(bf16)
            return f

        def ff2(u):
            def f():
                cols = slice(u * SUB, (u + 1) * SUB)
                x2 = st["x1", u] + jnp.dot(w2t_v[...], st["h", u], preferred_element_type=f32)
                xres[b, :, cols] = x2
                outb[b, :, cols] = x2.astype(bf16)
            return f
        return ([proj(u) for u in range(NSUB)] + [ff1(u) for u in range(NSUB)] + [ff2(u) for u in range(NSUB)])

    def out_copy(b):
        c0 = b * TB
        if not isinstance(b, int):
            c0 = pl.multiple_of(c0, TB)
        return pltpu.make_async_copy(outb.at[b], out_hbm.at[0, :, pl.ds(c0, TB)], sem_out.at[b])

    def layer(l, carry):
        p1(l)
        for f in a_items(0, sbuf[0], mbuf[0]):
            f()

        @pl.when(l == 0)
        def _():
            for cp in late:
                cp.wait()
            w = wo_v[...]
            parts = []
            for h in range(H):
                parts += [w[h * DH:(h + 1) * DH, :], zpad]
            wo_t[...] = jnp.concatenate(parts, axis=0).T

        attn_loop()

        lb = (NT - 1) % 3
        bi = b_items(NT - 1, sbuf[lb], mbuf[lb])
        di = dense_items(0)
        half = NCB // 2
        di[0]()
        for f in bi[:half]:
            f()
        di[1]()
        for f in bi[half:]:
            f()
        for f in di[2:]:
            f()

        @pl.when(l == 1)
        def _():
            out_copy(0).start()

        def dbody(b, c):
            for f in dense_items(b):
                f()

            @pl.when(l == 1)
            def _():
                out_copy(b).start()
            return c
        lax.fori_loop(1, NB, dbody, 0)
        return carry

    lax.fori_loop(0, 2, layer, 0)
    for b in range(NB):
        out_copy(b).wait()


@jax.jit
def pallas_interleave_layers__grouped_kv_mqa__dense_activation_relu__prompt_kernel(
    A_x, A_wq, A_wk, A_wv, A_wo, B_x, B_w1, B_w2,
):
    del B_x
    hbm_spec = pl.BlockSpec(memory_space=pltpu.HBM)
    scratch = [
        pltpu.VMEM((NB, D, TB), bf16),
        pltpu.VMEM((D, D), bf16),
        pltpu.VMEM((DH, D), bf16),
        pltpu.VMEM((DH, D), bf16),
        pltpu.VMEM((D, D), bf16),
        pltpu.VMEM((D, DFF), bf16),
        pltpu.VMEM((D, DFF), bf16),
        pltpu.VMEM((NB, D, TB), f32),
        pltpu.VMEM((NQKV, D), bf16),
        pltpu.VMEM((D, NQ), bf16),
        pltpu.VMEM((DFF, D), bf16),
        pltpu.VMEM((S, DP), bf16),
        pltpu.VMEM((NB, NQ, TB), bf16),
        pltpu.VMEM((NB, DP, TB), bf16),
        pltpu.VMEM((NB, NQ, TB), bf16),
        pltpu.VMEM((S, TB), f32),
        pltpu.VMEM((S, TB), f32),
        pltpu.VMEM((S, TB), f32),
        pltpu.VMEM((8, TB), f32),
        pltpu.VMEM((8, TB), f32),
        pltpu.VMEM((8, TB), f32),
        pltpu.VMEM((NB, D, TB), bf16),
        pltpu.SemaphoreType.DMA((6,)),
        pltpu.SemaphoreType.DMA((NB,)),
        pltpu.SemaphoreType.DMA((NB,)),
    ]
    out_t = pl.pallas_call(
        _kernel,
        out_shape=jax.ShapeDtypeStruct((1, D, S), A_x.dtype),
        in_specs=[hbm_spec] * 7,
        out_specs=hbm_spec,
        scratch_shapes=scratch,
        compiler_params=pltpu.CompilerParams(vmem_limit_bytes=100 * 1024 * 1024),
        name="fused_layers",
    )(jnp.transpose(A_x, (0, 2, 1)), A_wq, A_wk.T, A_wv.T, A_wo, B_w1, B_w2.T)
    return jnp.transpose(out_t, (0, 2, 1))
```

```python
import functools
import math

import jax
import jax.numpy as jnp
from jax import lax
from jax.experimental import pallas as pl
from jax.experimental.pallas import tpu as pltpu

f32 = jnp.float32
bf16 = jnp.bfloat16

S = 2048
D = 448
H = 16
DH = 28
DP = 32
DFF = 1792
TB = 512
NB = S // TB
CKA = 128
CKB = 256
NCA = S // CKA
NCB = S // CKB
NT = H * NB
TPB = 9
SUB = 256
NSUB = TB // SUB
EPS = 1e-5
INITLOOP = 0
BSTEP = 192
LPOS = (1, 3)
LASTW = 768
SKEW = 256
QSCALE = (DH ** -0.5) * math.log2(math.e)
NQ = H * DP
NQKV = D + 2 * DP
NIT = (NT - 1) // TPB
W1C = -(-(DFF // 128) // NIT) * 128

NT_DIMS = (((1,), (1,)), ((), ()))


def _sum0(x):
    parts = [x[i:i + 8] for i in range(0, x.shape[0], 8)]
    while len(parts) > 1:
        nxt = [parts[i] + parts[i + 1] for i in range(0, len(parts) - 1, 2)]
        if len(parts) % 2:
            nxt.append(parts[-1])
        parts = nxt
    return jnp.sum(parts[0], axis=0, keepdims=True)


def _ln_t(x):
    mu = jnp.mean(x, axis=0, keepdims=True)
    xc = x - mu
    var = jnp.mean(xc * xc, axis=0, keepdims=True)
    return (xc * lax.rsqrt(var + EPS)).astype(bf16)


def _tree_max8(s):
    r = s.shape[0]
    while r > 8:
        r //= 2
        s = jnp.maximum(s[:r], s[r:])
    return s


def _kernel(x_hbm, wq_hbm, wkt_hbm, wvt_hbm, wo_hbm, w1_hbm, w2t_hbm, out_hbm,
            xin, wq_v, wkt_v, wvt_v, wo_v, w1_v, w2t_v,
            xres, wqkv_t, wo_t, w1_t, k_s, qt_s, vt_s, ot_s, s0, s1, s2, m0, m1, m2, acc_s, outb,
            sem_in, sem_x, sem_out):
    sbuf = (s0, s1, s2)
    mbuf = (m0, m1, m2)
    early = []
    for i, (src, dst) in enumerate([(wq_hbm, wq_v), (wkt_hbm, wkt_v), (wvt_hbm, wvt_v)]):
        cp = pltpu.make_async_copy(src, dst, sem_in.at[i]); cp.start(); early.append(cp)
    xcps = [pltpu.make_async_copy(x_hbm.at[0, :, pl.ds(b * TB, TB)], xin.at[b], sem_x.at[b]) for b in range(NB)]
    xcps[0].start()
    late = [pltpu.make_async_copy(wo_hbm, wo_v, sem_in.at[3]),
            pltpu.make_async_copy(w1_hbm, w1_v, sem_in.at[4]),
            pltpu.make_async_copy(w2t_hbm, w2t_v, sem_in.at[5])]

    for cp in early:
        cp.wait()
    for cp in xcps[1:]:
        cp.start()
    wqkv_t[0:D, :] = wq_v[...].T
    zpad = jnp.zeros((DP - DH, D), bf16)
    wqkv_t[D:D + DP, :] = jnp.concatenate([wvt_v[...], zpad], axis=0)
    wqkv_t[D + DP:NQKV, :] = jnp.concatenate([wkt_v[...], zpad], axis=0)

    def p1(blocks, first):
        for b in blocks:
            for u in range(NSUB):
                cols = slice(u * SUB, (u + 1) * SUB)
                if first:
                    xs = xin[b, :, cols].astype(f32)
                    xres[b, :, cols] = xs
                else:
                    xs = xres[b, :, cols]
                qkv_sub(b, u, xs)

    def qkv_sub(b, u, xs):
        cols = slice(u * SUB, (u + 1) * SUB)
        xn = _ln_t(xs)
        qkv = jnp.dot(wqkv_t[...], xn, preferred_element_type=f32)
        for h in range(H):
            qt_s[b, h * DP:(h + 1) * DP, cols] = (qkv[h * DH:h * DH + DP] * QSCALE).astype(bf16)
        v = qkv[D:D + DP]
        rr = lax.broadcasted_iota(jnp.int32, (DP, SUB), 0)
        v = jnp.where(rr == DH, 1.0, v)
        row0 = b * TB + u * SUB
        if not isinstance(row0, int):
            row0 = pl.multiple_of(row0, SUB)
        vt_s[:, pl.ds(row0, SUB)] = v.astype(bf16)
        k_s[pl.ds(row0, SUB), :] = qkv[D + DP:].T.astype(bf16)

    def idx(t):
        return t % H, t // H

    def a_items(ta, sa, ma):
        st = {}

        def chunk(c):
            def f():
                if c == 0:
                    ha, qa = idx(ta)
                    st["w"] = qt_s[qa, pl.ds(pl.multiple_of(ha * DP, DP), DP), :]
                s = jnp.dot(k_s[c * CKA:(c + 1) * CKA, :], st["w"], preferred_element_type=f32)
                sa[c * CKA:(c + 1) * CKA, :] = s
                mc = _tree_max8(s)
                st["m"] = mc if c == 0 else jnp.maximum(st["m"], mc)
                if c == NCA - 1:
                    ma[...] = jnp.broadcast_to(jnp.max(st["m"], axis=0, keepdims=True), (8, TB))
            return f
        return [chunk(c) for c in range(NCA)]

    def b_items(tb, sb, mb):
        st = {}

        def chunk(c):
            def f():
                if c == 0:
                    st["m"] = mb[0:1, :]
                p = jnp.exp2(sb[c * CKB:(c + 1) * CKB, :] - st["m"]).astype(bf16)
                d = jnp.dot(vt_s[:, c * CKB:(c + 1) * CKB], p, preferred_element_type=f32)
                st["acc"] = d if c == 0 else st["acc"] + d
                if c == NCB - 1:
                    hb, qb = idx(tb)
                    acc = st["acc"]
                    inv = 1.0 / acc[DH:DH + 1, :]
                    ot_s[qb, pl.ds(pl.multiple_of(hb * DP, DP), DP), :] = (acc * inv).astype(bf16)
            return f
        return [chunk(c) for c in range(NCB)]

    def last_items(b):
        st = {}
        tl = NT - 1
        sl, ml = sbuf[tl % 3], mbuf[tl % 3]
        lo = b * LASTW
        k0 = jnp.minimum(lo, S - LASTW)
        nch = LASTW // CKB

        def chunk(c):
            def f():
                r0 = pl.multiple_of(k0 + c * CKB, 128)
                p = jnp.exp2(sl[pl.ds(r0, CKB), :] - ml[0:1, :])
                rows = lax.broadcasted_iota(jnp.int32, (CKB, TB), 0)
                p = jnp.where(rows >= lo - r0, p, 0.0).astype(bf16)
                d = jnp.dot(vt_s[:, pl.ds(r0, CKB)], p, preferred_element_type=f32)
                st["acc"] = (acc_s[...] if c == 0 else st["acc"]) + d
                if c == nch - 1:
                    acc = st["acc"]
                    acc_s[...] = acc
                    inv = 1.0 / jnp.maximum(acc[DH:DH + 1, :], 1e-30)
                    hl, ql = tl % H, tl // H
                    ot_s[ql, hl * DP:(hl + 1) * DP, :] = (acc * inv).astype(bf16)
            return f
        return [chunk(c) for c in range(nch)]

    def wo_prep():
        w = wo_v[...]
        parts = []
        for h in range(H):
            parts += [w[h * DH:(h + 1) * DH, :], jnp.zeros((DP - DH, D), bf16)]
        wo_t[...] = jnp.concatenate(parts, axis=0).T

    def attn_loop():
        def body(j, carry):
            ai, bi = [], []
            for u in range(TPB):
                t = TPB * j + u
                ai += a_items(t + 1, sbuf[(u + 1) % 3], mbuf[(u + 1) % 3])
                bi += b_items(t, sbuf[u % 3], mbuf[u % 3])
            seq = [(i * CKA, 0, f) for i, f in enumerate(ai)] + [((i // NCB) * S + SKEW + (i % NCB) * BSTEP, 1, f) for i, f in enumerate(bi)]
            for _, _, f in sorted(seq, key=lambda e: e[:2]):
                f()
            c0 = pl.multiple_of(jnp.minimum(j * W1C, DFF - W1C), 128)
            w1_t[pl.ds(c0, W1C), :] = w1_v[:, pl.ds(c0, W1C)].T
            wo_prep()
            return carry
        lax.fori_loop(0, NIT, body, 0)

    def dense_items(b):
        st = {}

        def proj(u):
            def f():
                cols = slice(u * SUB, (u + 1) * SUB)
                o = jnp.dot(wo_t[...], ot_s[b, :, cols], preferred_element_type=f32)
                st["x1", u] = xres[b, :, cols] + o
            return f

        def ff1(u):
            def f():
                st["h", u] = jnp.maximum(
                    jnp.dot(w1_t[...], _ln_t(st["x1", u]), preferred_element_type=f32), 0.0).astype(bf16)
            return f

        def ff2(u):
            def f():
                cols = slice(u * SUB, (u + 1) * SUB)
                x2 = st["x1", u] + jnp.dot(w2t_v[...], st["h", u], preferred_element_type=f32)
                xres[b, :, cols] = x2
                outb[b, :, cols] = x2.astype(bf16)
            return f
        return ([proj(u) for u in range(NSUB)] + [ff1(u) for u in range(NSUB)] + [ff2(u) for u in range(NSUB)])

    def out_copy(b):
        c0 = b * TB
        if not isinstance(b, int):
            c0 = pl.multiple_of(c0, TB)
        return pltpu.make_async_copy(outb.at[b], out_hbm.at[0, :, pl.ds(c0, TB)], sem_out.at[b])

    def layer(l, carry):
        attn_loop()

        acc_s[...] = jnp.zeros((DP, TB), f32)

        def dbody(b, c):
            di = dense_items(b)
            li = last_items(b)
            nb = 0
            for i, f in enumerate(di):
                f()
                upto = LPOS[i] if i < len(LPOS) else len(li)
                while nb < upto:
                    li[nb]()
                    nb += 1

            @pl.when(l == 1)
            def _():
                out_copy(b).start()
            return c
        lax.fori_loop(0, NB, dbody, 0)

        @pl.when(l == 0)
        def _():
            p1(range(NB), False)
            for f in a_items(0, sbuf[0], mbuf[0]):
                f()
        return carry

    xcps[0].wait()
    p1(range(0, 1), True)
    for cp in xcps[1:]:
        cp.wait()
    for cp in late:
        cp.start()
    if INITLOOP:
        def p1_body(b, c):
            p1([b], True)
            return c
        lax.fori_loop(1, INITLOOP + 1, p1_body, 0)
    p1(range(1 + INITLOOP, NB), True)
    for f in a_items(0, sbuf[0], mbuf[0]):
        f()
    for cp in late:
        cp.wait()

    lax.fori_loop(0, 2, layer, 0)
    for b in range(NB):
        out_copy(b).wait()


@jax.jit
def pallas_interleave_layers__grouped_kv_mqa__dense_activation_relu__prompt_kernel(
    A_x, A_wq, A_wk, A_wv, A_wo, B_x, B_w1, B_w2,
):
    del B_x
    hbm_spec = pl.BlockSpec(memory_space=pltpu.HBM)
    scratch = [
        pltpu.VMEM((NB, D, TB), bf16),
        pltpu.VMEM((D, D), bf16),
        pltpu.VMEM((DH, D), bf16),
        pltpu.VMEM((DH, D), bf16),
        pltpu.VMEM((D, D), bf16),
        pltpu.VMEM((D, DFF), bf16),
        pltpu.VMEM((D, DFF), bf16),
        pltpu.VMEM((NB, D, TB), f32),
        pltpu.VMEM((NQKV, D), bf16),
        pltpu.VMEM((D, NQ), bf16),
        pltpu.VMEM((DFF, D), bf16),
        pltpu.VMEM((S, DP), bf16),
        pltpu.VMEM((NB, NQ, TB), bf16),
        pltpu.VMEM((DP, S), bf16),
        pltpu.VMEM((NB, NQ, TB), bf16),
        pltpu.VMEM((S, TB), f32),
        pltpu.VMEM((S, TB), f32),
        pltpu.VMEM((S, TB), f32),
        pltpu.VMEM((8, TB), f32),
        pltpu.VMEM((8, TB), f32),
        pltpu.VMEM((8, TB), f32),
        pltpu.VMEM((DP, TB), f32),
        pltpu.VMEM((NB, D, TB), bf16),
        pltpu.SemaphoreType.DMA((6,)),
        pltpu.SemaphoreType.DMA((NB,)),
        pltpu.SemaphoreType.DMA((NB,)),
    ]
    out_t = pl.pallas_call(
        _kernel,
        out_shape=jax.ShapeDtypeStruct((1, D, S), A_x.dtype),
        in_specs=[hbm_spec] * 7,
        out_specs=hbm_spec,
        scratch_shapes=scratch,
        compiler_params=pltpu.CompilerParams(vmem_limit_bytes=100 * 1024 * 1024),
        name="fused_layers",
    )(jnp.transpose(A_x, (0, 2, 1)), A_wq, A_wk.T, A_wv.T, A_wo, B_w1, B_w2.T)
    return jnp.transpose(out_t, (0, 2, 1))
```

```python
import math

import jax
import jax.numpy as jnp
from jax import lax
from jax.experimental import pallas as pl
from jax.experimental.pallas import tpu as pltpu

f32 = jnp.float32
bf16 = jnp.bfloat16

S = 2048
D = 448
H = 16
DH = 28
DP = 32
DFF = 1792
EPS = 1e-5
TB = 512
NB = S // TB
SUB = 256
NSUB = TB // SUB
CKA = 128
CKB = 256
NCA = S // CKA
NCB = S // CKB
NT = H * NB
TPB = 9
NIT = (NT - 1) // TPB
SKEW = 256
BSTEP = 192
LASTW = 768
QSCALE = (DH ** -0.5) * math.log2(math.e)
NQ = H * DP
NQKV = D + 2 * DP
W1C = -(-(DFF // 128) // NIT) * 128


def _ln_t(x):
    mu = jnp.mean(x, axis=0, keepdims=True)
    xc = x - mu
    var = jnp.mean(xc * xc, axis=0, keepdims=True)
    return (xc * lax.rsqrt(var + EPS)).astype(bf16)


def _tree_max8(s):
    r = s.shape[0]
    while r > 8:
        r //= 2
        s = jnp.maximum(s[:r], s[r:])
    return s


def _kernel(x_hbm, wq_hbm, wkt_hbm, wvt_hbm, wo_hbm, w1_hbm, w2t_hbm, out_hbm,
            xin, wq_v, wkt_v, wvt_v, wo_v, w1_v, w2t_v,
            xres, wqkv_t, wo_t, w1_t, k_s, qt_s, vt_s, ot_s, s0, s1, s2, m0, m1, m2, acc_s, outb,
            sem_in, sem_x, sem_out):
    sbuf = (s0, s1, s2)
    mbuf = (m0, m1, m2)

    early = [pltpu.make_async_copy(src, dst, sem_in.at[i])
             for i, (src, dst) in enumerate([(wq_hbm, wq_v), (wkt_hbm, wkt_v), (wvt_hbm, wvt_v)])]
    late = [pltpu.make_async_copy(src, dst, sem_in.at[3 + i])
            for i, (src, dst) in enumerate([(wo_hbm, wo_v), (w1_hbm, w1_v), (w2t_hbm, w2t_v)])]
    xcps = [pltpu.make_async_copy(x_hbm.at[0, :, pl.ds(b * TB, TB)], xin.at[b], sem_x.at[b]) for b in range(NB)]

    def out_copy(b):
        c0 = b * TB if isinstance(b, int) else pl.multiple_of(b * TB, TB)
        return pltpu.make_async_copy(outb.at[b], out_hbm.at[0, :, pl.ds(c0, TB)], sem_out.at[b])

    def qkv_sub(b, u, xs):
        cols = slice(u * SUB, (u + 1) * SUB)
        qkv = jnp.dot(wqkv_t[...], _ln_t(xs), preferred_element_type=f32)
        for h in range(H):
            qt_s[b, h * DP:(h + 1) * DP, cols] = (qkv[h * DH:h * DH + DP] * QSCALE).astype(bf16)
        rr = lax.broadcasted_iota(jnp.int32, (DP, SUB), 0)
        v = jnp.where(rr == DH, 1.0, qkv[D:D + DP])
        tok0 = b * TB + u * SUB
        vt_s[:, tok0:tok0 + SUB] = v.astype(bf16)
        k_s[tok0:tok0 + SUB, :] = qkv[D + DP:].T.astype(bf16)

    def projections(blocks, first):
        for b in blocks:
            for u in range(NSUB):
                cols = slice(u * SUB, (u + 1) * SUB)
                if first:
                    xs = xin[b, :, cols].astype(f32)
                    xres[b, :, cols] = xs
                else:
                    xs = xres[b, :, cols]
                qkv_sub(b, u, xs)

    def a_items(t, s_ref, m_ref):
        st = {}

        def chunk(c):
            def emit():
                if c == 0:
                    st["w"] = qt_s[t // H, pl.ds(pl.multiple_of((t % H) * DP, DP), DP), :]
                s = jnp.dot(k_s[c * CKA:(c + 1) * CKA, :], st["w"], preferred_element_type=f32)
                s_ref[c * CKA:(c + 1) * CKA, :] = s
                mc = _tree_max8(s)
                st["m"] = mc if c == 0 else jnp.maximum(st["m"], mc)
                if c == NCA - 1:
                    m_ref[...] = jnp.broadcast_to(jnp.max(st["m"], axis=0, keepdims=True), (8, TB))
            return emit
        return [chunk(c) for c in range(NCA)]

    def b_items(t, s_ref, m_ref):
        st = {}

        def chunk(c):
            def emit():
                if c == 0:
                    st["m"] = m_ref[0:1, :]
                p = jnp.exp2(s_ref[c * CKB:(c + 1) * CKB, :] - st["m"]).astype(bf16)
                d = jnp.dot(vt_s[:, c * CKB:(c + 1) * CKB], p, preferred_element_type=f32)
                st["acc"] = d if c == 0 else st["acc"] + d
                if c == NCB - 1:
                    acc = st["acc"]
                    inv = 1.0 / acc[DH:DH + 1, :]
                    ot_s[t // H, pl.ds(pl.multiple_of((t % H) * DP, DP), DP), :] = (acc * inv).astype(bf16)
            return emit
        return [chunk(c) for c in range(NCB)]

    def last_items(b):
        st = {}
        t = NT - 1
        s_ref, m_ref = sbuf[t % 3], mbuf[t % 3]
        lo = b * LASTW
        k0 = jnp.minimum(lo, S - LASTW)
        nch = LASTW // CKB

        def chunk(c):
            def emit():
                r0 = pl.multiple_of(k0 + c * CKB, CKB)
                p = jnp.exp2(s_ref[pl.ds(r0, CKB), :] - m_ref[0:1, :])
                rows = lax.broadcasted_iota(jnp.int32, (CKB, TB), 0)
                p = jnp.where(rows >= lo - r0, p, 0.0).astype(bf16)
                d = jnp.dot(vt_s[:, pl.ds(r0, CKB)], p, preferred_element_type=f32)
                st["acc"] = (acc_s[...] if c == 0 else st["acc"]) + d
                if c == nch - 1:
                    acc = st["acc"]
                    acc_s[...] = acc
                    inv = 1.0 / jnp.maximum(acc[DH:DH + 1, :], 1e-30)
                    ot_s[t // H, (t % H) * DP:(t % H + 1) * DP, :] = (acc * inv).astype(bf16)
            return emit
        return [chunk(c) for c in range(nch)]

    def scores_of_first_tile():
        for emit in a_items(0, sbuf[0], mbuf[0]):
            emit()

    def attention_loop():
        def body(j, carry):
            ai, bi = [], []
            for u in range(TPB):
                t = TPB * j + u
                ai += a_items(t + 1, sbuf[(u + 1) % 3], mbuf[(u + 1) % 3])
                bi += b_items(t, sbuf[u % 3], mbuf[u % 3])
            seq = [(i * CKA, 0, e) for i, e in enumerate(ai)]
            seq += [((i // NCB) * S + SKEW + (i % NCB) * BSTEP, 1, e) for i, e in enumerate(bi)]
            for _, _, emit in sorted(seq, key=lambda e: e[:2]):
                emit()
            c0 = pl.multiple_of(jnp.minimum(j * W1C, DFF - W1C), 128)
            w1_t[pl.ds(c0, W1C), :] = w1_v[:, pl.ds(c0, W1C)].T
            wo = wo_v[...]
            parts = []
            for h in range(H):
                parts += [wo[h * DH:(h + 1) * DH, :], jnp.zeros((DP - DH, D), bf16)]
            wo_t[...] = jnp.concatenate(parts, axis=0).T
            return carry
        lax.fori_loop(0, NIT, body, 0)

    def dense_items(b):
        st = {}

        def proj(u):
            def emit():
                cols = slice(u * SUB, (u + 1) * SUB)
                o = jnp.dot(wo_t[...], ot_s[b, :, cols], preferred_element_type=f32)
                st["x1", u] = xres[b, :, cols] + o
            return emit

        def ff1(u):
            def emit():
                h = jnp.dot(w1_t[...], _ln_t(st["x1", u]), preferred_element_type=f32)
                st["h", u] = jnp.maximum(h, 0.0).astype(bf16)
            return emit

        def ff2(u):
            def emit():
                cols = slice(u * SUB, (u + 1) * SUB)
                x2 = st["x1", u] + jnp.dot(w2t_v[...], st["h", u], preferred_element_type=f32)
                xres[b, :, cols] = x2
                outb[b, :, cols] = x2.astype(bf16)
            return emit
        return [f(u) for f in (proj, ff1, ff2) for u in range(NSUB)]

    def layer(l, carry):
        attention_loop()
        acc_s[...] = jnp.zeros((DP, TB), f32)

        def dense_body(b, c):
            di, li = dense_items(b), last_items(b)
            for i, emit in enumerate(di):
                emit()
                if 1 <= i <= len(li):
                    li[i - 1]()

            @pl.when(l == 1)
            def _():
                out_copy(b).start()
            return c
        lax.fori_loop(0, NB, dense_body, 0)

        @pl.when(l == 0)
        def _():
            projections(range(NB), False)
            scores_of_first_tile()
        return carry

    for cp in early:
        cp.start()
    xcps[0].start()
    for cp in early:
        cp.wait()
    for cp in xcps[1:]:
        cp.start()
    zpad = jnp.zeros((DP - DH, D), bf16)
    wqkv_t[0:D, :] = wq_v[...].T
    wqkv_t[D:D + DP, :] = jnp.concatenate([wvt_v[...], zpad], axis=0)
    wqkv_t[D + DP:NQKV, :] = jnp.concatenate([wkt_v[...], zpad], axis=0)

    xcps[0].wait()
    projections([0], True)
    for cp in xcps[1:]:
        cp.wait()
    for cp in late:
        cp.start()
    projections(range(1, NB), True)
    scores_of_first_tile()
    for cp in late:
        cp.wait()

    lax.fori_loop(0, 2, layer, 0)

    for b in range(NB):
        out_copy(b).wait()


@jax.jit
def pallas_interleave_layers__grouped_kv_mqa__dense_activation_relu__prompt_kernel(
    A_x, A_wq, A_wk, A_wv, A_wo, B_x, B_w1, B_w2,
):
    del B_x
    hbm = pl.BlockSpec(memory_space=pltpu.HBM)
    scratch = [
        pltpu.VMEM((NB, D, TB), bf16),
        pltpu.VMEM((D, D), bf16),
        pltpu.VMEM((DH, D), bf16),
        pltpu.VMEM((DH, D), bf16),
        pltpu.VMEM((D, D), bf16),
        pltpu.VMEM((D, DFF), bf16),
        pltpu.VMEM((D, DFF), bf16),
        pltpu.VMEM((NB, D, TB), f32),
        pltpu.VMEM((NQKV, D), bf16),
        pltpu.VMEM((D, NQ), bf16),
        pltpu.VMEM((DFF, D), bf16),
        pltpu.VMEM((S, DP), bf16),
        pltpu.VMEM((NB, NQ, TB), bf16),
        pltpu.VMEM((DP, S), bf16),
        pltpu.VMEM((NB, NQ, TB), bf16),
        pltpu.VMEM((S, TB), f32),
        pltpu.VMEM((S, TB), f32),
        pltpu.VMEM((S, TB), f32),
        pltpu.VMEM((8, TB), f32),
        pltpu.VMEM((8, TB), f32),
        pltpu.VMEM((8, TB), f32),
        pltpu.VMEM((DP, TB), f32),
        pltpu.VMEM((NB, D, TB), bf16),
        pltpu.SemaphoreType.DMA((6,)),
        pltpu.SemaphoreType.DMA((NB,)),
        pltpu.SemaphoreType.DMA((NB,)),
    ]
    out_t = pl.pallas_call(
        _kernel,
        out_shape=jax.ShapeDtypeStruct((1, D, S), A_x.dtype),
        in_specs=[hbm] * 7,
        out_specs=hbm,
        scratch_shapes=scratch,
        compiler_params=pltpu.CompilerParams(vmem_limit_bytes=64 * 1024 * 1024),
        name="fused_layers",
    )(jnp.transpose(A_x, (0, 2, 1)), A_wq, A_wk.T, A_wv.T, A_wo, B_w1, B_w2.T)
    return jnp.transpose(out_t, (0, 2, 1))
```
